```python
import jax
import jax.numpy as jnp

def _softmax(x, axis=-1):
    return jax.nn.softmax(x, axis=axis)
def _gelu(x):
    return jax.nn.gelu(x, approximate=True)
def _silu(x):
    return jax.nn.silu(x)
def _sigmoid(x):
    return jax.nn.sigmoid(x)
def _layernorm(x, axis=-1, eps=1e-5):
    m = jnp.mean(x, axis=axis, keepdims=True)
    v = jnp.var(x, axis=axis, keepdims=True)
    return (x - m) / jnp.sqrt(v + eps)
def _scatter_add(tgt, idx, src, axis=0):
    return tgt.at[idx].add(src)
def _segment_sum(src, seg, n):
    return jax.ops.segment_sum(src, seg, n)
class _Rng:
    def __init__(self, key):
        self._k = key
    def _next(self):
        self._k, sub = jax.random.split(self._k)
        return sub
    def normal(self, shape):
        return jax.random.normal(self._next(), shape, dtype=jnp.bfloat16)
    def randint(self, lo, hi, shape):
        return jax.random.randint(self._next(), shape, lo, hi, dtype=jnp.int32)
    def uniform(self, shape, lo=0.0, hi=1.0):
        return jax.random.uniform(self._next(), shape, jnp.bfloat16, lo, hi)
    def permutation(self, n):
        return jax.random.permutation(self._next(), n)


kernel_name = 'parallel_sum__gqa_block_cached__moe_arch_mod__decode'

def setup_inputs():
    _rng = _Rng(jax.random.key(int.from_bytes(__import__("os").urandom(4), "little")))
    _w = (lambda a: (lambda t: t.astype(jnp.bfloat16) if jnp.issubdtype(t.dtype, jnp.floating) else t)(jnp.asarray(a)))
    def _A_setup():
        B, Sq, D = 1, 1, 448
        Hq, Hkv, Sk, Dh = 16, 8, 65536, 256
        assert Hq % Hkv == 0, (Hq, Hkv)
        return {
            "x": _w((lambda *s: _rng.normal(s) * 0.05)(B, Sq, D)),
            "k_cache": _w((lambda *s: _rng.normal(s) * 0.05)(B, Hkv, Sk, Dh)),
            "v_cache": _w((lambda *s: _rng.normal(s) * 0.05)(B, Hkv, Sk, Dh)),
            "wq": _w((lambda *s: _rng.normal(s) * 0.05)(D, Hq * Dh) * (D ** -0.5)),
            "wo": _w((lambda *s: _rng.normal(s) * 0.05)(Hq * Dh, D) * ((Hq * Dh) ** -0.5)),
        }
    _A_in = _A_setup()

    def _B_setup():
        B, S, D, F, C = 1, 1, 448, 1792, 1
        return {
            "x": _w((lambda *s: _rng.normal(s) * 0.05)(B, S, D)),
            "w_r": _w((lambda *s: _rng.normal(s) * 0.05)(D)),
            "w_gate": _w((lambda *s: _rng.normal(s) * 0.05)(D, F)),
            "w_up": _w((lambda *s: _rng.normal(s) * 0.05)(D, F)),
            "w_down": _w((lambda *s: _rng.normal(s) * 0.05)(F, D)),
        }
    _B_in = _B_setup()

    return {
        "A_x": _A_in["x"],
        "A_k_cache": _A_in["k_cache"],
        "A_v_cache": _A_in["v_cache"],
        "A_wq": _A_in["wq"],
        "A_wo": _A_in["wo"],
        "B_x": _B_in["x"],
        "B_w_r": _B_in["w_r"],
        "B_w_gate": _B_in["w_gate"],
        "B_w_up": _B_in["w_up"],
        "B_w_down": _B_in["w_down"],
    }

def reference(A_x, A_k_cache, A_v_cache, A_wq, A_wo, B_x, B_w_r, B_w_gate, B_w_up, B_w_down):
    def _A_ref(x, k_cache, v_cache, wq, wo):
        B, Sq, D = x.shape
        Hq, Dh = 16, 256
        Hkv = k_cache.shape[1]
        rep = Hq // Hkv
        q = (lambda x, *d: x.transpose(*d))((x @ wq).reshape(B, Sq, Hq, Dh), 0, 2, 1, 3)
        k = jnp.repeat(k_cache, rep, axis=1)
        v = jnp.repeat(v_cache, rep, axis=1)
        scores = jnp.einsum("bhqd,bhkd->bhqk", q, k) * (Dh ** -0.5)
        p = _softmax(scores, axis=-1)
        o = jnp.einsum("bhqk,bhkd->bhqd", p, v)
        return (lambda x, *d: x.transpose(*d))(o, 0, 2, 1, 3).reshape(B, Sq, Hq * Dh) @ wo

    def _B_ref(x, w_r, w_gate, w_up, w_down):
        B, S, D = x.shape
        C = 1
        r = x @ w_r
        idx = jnp.argsort(-r, axis=-1)[:, :C]
        idx_e = jnp.repeat(idx.reshape(B, C, 1), D, axis=2)
        x_sel = jnp.take_along_axis(x, idx_e, axis=1)
        g = _silu(x_sel @ w_gate)
        u = x_sel @ w_up
        y = (g * u) @ w_down
        r_sel = _sigmoid(jnp.take_along_axis(r, idx, axis=1))
        y = y * r_sel.reshape(B, C, 1)
        b_off = (jnp.arange(B) * S).reshape(B, 1)
        flat_idx = (idx + b_off).reshape(B * C)
        zero = (x * 0.0).reshape(B * S, D)
        upd = _scatter_add(zero, flat_idx, y.reshape(B * C, D), axis=0)
        return x + upd.reshape(B, S, D)

    x = A_x
    xn = _layernorm(x, axis=-1)
    return x + _A_ref(xn, A_k_cache, A_v_cache, A_wq, A_wo) + _B_ref(xn, B_w_r, B_w_gate, B_w_up, B_w_down)
```

```python
import jax
import jax.numpy as jnp
from jax.experimental import pallas as pl
from jax.experimental.pallas import tpu as pltpu

HQ, DH = 16, 256
NT = (((1,), (1,)), ((), ()))

T = 1024
NBUF = 4
TS = 64
F32, BF16 = jnp.float32, jnp.bfloat16


def _kernel(x_hbm, wr_hbm, k_hbm, v_hbm, wq_hbm, wot_hbm, wg_hbm, wu_hbm, wdt_hbm, out_ref,
            kbuf, vbuf, x_v, wr_v, wq_v, wot_v, wg_v, wu_v, wdt_v, q_s, ksem, vsem, wsem):
    _, hkv, sk, _ = k_hbm.shape
    d = x_hbm.shape[-1]
    nc = sk // T
    total = hkv * nc
    rep = HQ // hkv
    assert rep == 2 and sk % T == 0 and total >= NBUF

    def issue(i, slot):
        h = i // nc
        c = i % nc
        for j in range(T // TS):
            r0 = pl.multiple_of(c * T + j * TS, TS)
            pltpu.make_async_copy(k_hbm.at[0, h, pl.ds(r0, TS), :],
                                  kbuf.at[slot, pl.ds(j * TS, TS), :], ksem.at[slot]).start(priority=0)
            pltpu.make_async_copy(v_hbm.at[0, h, pl.ds(r0, TS), :],
                                  vbuf.at[slot, pl.ds(j * TS, TS), :], vsem.at[slot]).start(priority=1)

    def wait_all(buf, sem):
        pltpu.make_async_copy(buf, buf, sem).wait()

    cx = pltpu.make_async_copy(x_hbm, x_v, wsem.at[5])
    cr = pltpu.make_async_copy(wr_hbm, wr_v, wsem.at[6])
    cq = pltpu.make_async_copy(wq_hbm, wq_v, wsem.at[0])
    co = pltpu.make_async_copy(wot_hbm, wot_v, wsem.at[1])
    cg = pltpu.make_async_copy(wg_hbm, wg_v, wsem.at[2])
    cu = pltpu.make_async_copy(wu_hbm, wu_v, wsem.at[3])
    cd = pltpu.make_async_copy(wdt_hbm, wdt_v, wsem.at[4])
    cx.start()
    cr.start()
    cq.start()
    for s in range(NBUF):
        issue(s, s)
        if s == 0:
            cg.start()
            cu.start()
            cd.start()
        if s == 1:
            co.start()

    cx.wait()
    x = x_v[0].astype(F32)
    mu = jnp.mean(x, axis=-1, keepdims=True)
    xc = x - mu
    var = jnp.mean(xc * xc, axis=-1, keepdims=True)
    xn = (xc * jax.lax.rsqrt(var + 1e-5)).astype(BF16).astype(F32)
    xn8 = jnp.broadcast_to(xn, (8, d)).astype(BF16)

    cq.wait()
    q = jnp.dot(xn8, wq_v[...], preferred_element_type=F32)
    q = q.astype(BF16).astype(F32) * (DH ** -0.5)
    row = jax.lax.broadcasted_iota(jnp.int32, (8, DH), 0)
    for g in range(hkv):
        qa = q[:, (2 * g) * DH:(2 * g + 1) * DH]
        qb = q[:, (2 * g + 1) * DH:(2 * g + 2) * DH]
        q_s[g] = jnp.where(row == 0, qa, qb)

    cg.wait()
    cu.wait()
    gate = jnp.dot(xn8, wg_v[...], preferred_element_type=F32).astype(BF16).astype(F32)
    up = jnp.dot(xn8, wu_v[...], preferred_element_type=F32).astype(BF16).astype(F32)
    hmid = (gate * jax.nn.sigmoid(gate) * up).astype(BF16)
    cd.wait()
    y = jax.lax.dot_general(hmid, wdt_v[...], NT, preferred_element_type=F32)[0:1]
    cr.wait()
    wr = wr_v[...].astype(F32).reshape(1, d)
    r = jnp.sum(xn * wr, axis=-1, keepdims=True)
    base = x + (xn + y * jax.nn.sigmoid(r))
    co.wait()

    def head_body(g, carry):
        acc_a, acc_b = carry
        qg = q_s[g].astype(BF16)

        def chunk_body(c, c2):
            m, l, acc = c2
            i = g * nc + c
            slot = i % NBUF
            wait_all(kbuf.at[slot], ksem.at[slot])
            s = jax.lax.dot_general(qg, kbuf[slot], NT, preferred_element_type=F32)
            m_new = jnp.maximum(m, jnp.max(s, axis=-1, keepdims=True))
            alpha = jnp.exp(m - m_new)
            p = jnp.exp(s - m_new)
            l = alpha * l + jnp.sum(p, axis=-1, keepdims=True)
            wait_all(vbuf.at[slot], vsem.at[slot])
            acc = alpha * acc + jnp.dot(p.astype(BF16), vbuf[slot], preferred_element_type=F32)

            @pl.when(i + NBUF < total)
            def _():
                issue(i + NBUF, slot)

            return m_new, l, acc

        m0 = jnp.full((8, 1), -jnp.inf, F32)
        l0 = jnp.zeros((8, 1), F32)
        a0 = jnp.zeros((8, DH), F32)
        _, l, acc = jax.lax.fori_loop(0, nc, chunk_body, (m0, l0, a0))
        o = (acc / l).astype(BF16)
        col = pl.multiple_of(g * (2 * DH), 2 * DH)
        acc_a = acc_a + jax.lax.dot_general(o, wot_v[:, pl.ds(col, DH)], NT, preferred_element_type=F32)
        acc_b = acc_b + jax.lax.dot_general(o, wot_v[:, pl.ds(col + DH, DH)], NT, preferred_element_type=F32)
        return acc_a, acc_b

    z = jnp.zeros((8, d), F32)
    acc_a, acc_b = jax.lax.fori_loop(0, hkv, head_body, (z, z))
    out_ref[0] = (base + (acc_a[0:1] + acc_b[1:2])).astype(out_ref.dtype)


@jax.jit
def pallas_parallel_sum__gqa_block_cached__moe_arch_mod__decode_kernel(
    A_x: jax.Array,
    A_k_cache: jax.Array,
    A_v_cache: jax.Array,
    A_wq: jax.Array,
    A_wo: jax.Array,
    B_x: jax.Array,
    B_w_r: jax.Array,
    B_w_gate: jax.Array,
    B_w_up: jax.Array,
    B_w_down: jax.Array,
):
    del B_x
    hkv = A_k_cache.shape[1]
    wot = A_wo.T
    wdt = B_w_down.T
    hbm = pl.BlockSpec(memory_space=pltpu.HBM)
    return pl.pallas_call(
        _kernel,
        out_shape=jax.ShapeDtypeStruct(A_x.shape, A_x.dtype),
        in_specs=[hbm] * 9,
        out_specs=pl.BlockSpec(memory_space=pltpu.VMEM),
        scratch_shapes=[
            pltpu.VMEM((NBUF, T, DH), BF16),
            pltpu.VMEM((NBUF, T, DH), BF16),
            pltpu.VMEM(A_x.shape, BF16),
            pltpu.VMEM(B_w_r.shape, BF16),
            pltpu.VMEM(A_wq.shape, BF16),
            pltpu.VMEM(wot.shape, BF16),
            pltpu.VMEM(B_w_gate.shape, BF16),
            pltpu.VMEM(B_w_up.shape, BF16),
            pltpu.VMEM(wdt.shape, BF16),
            pltpu.VMEM((hkv, 8, DH), F32),
            pltpu.SemaphoreType.DMA((NBUF,)),
            pltpu.SemaphoreType.DMA((NBUF,)),
            pltpu.SemaphoreType.DMA((7,)),
        ],
        compiler_params=pltpu.CompilerParams(vmem_limit_bytes=100 * 1024 * 1024),
    )(A_x, B_w_r, A_k_cache, A_v_cache, A_wq, wot, B_w_gate, B_w_up, wdt)
```

```python
import jax
import jax.numpy as jnp
from jax.experimental import pallas as pl
from jax.experimental.pallas import tpu as pltpu

HQ, DH = 16, 256
NT = (((1,), (1,)), ((), ()))

R = 2048
G = 4
TS = 16
ND = 16
TT = ND * TS
T = G * TT
NBUF = 4
F32, BF16 = jnp.float32, jnp.bfloat16


def _kernel(x_hbm, wr_hbm, k_hbm, v_hbm, wq_hbm, wot_hbm, wg_hbm, wu_hbm, wdt_hbm, out_ref,
            kbuf, vbuf, x_v, wr_v, wq_v, wot_v, wg_v, wu_v, wdt_v, q_s, ksem, vsem, wsem):
    hkv = q_s.shape[0]
    sk = k_hbm.shape[0] * R // hkv
    d = x_hbm.shape[-1]
    nc = sk // T
    nr = R // TT
    total = hkv * nc
    assert HQ == 2 * hkv and sk % (G * R) == 0 and total >= NBUF

    def issue(i, slot):
        b = pl.multiple_of((i // nr) * G, G)
        c = i % nr
        for j in range(ND):
            r0 = pl.multiple_of(c * TT + j * TS, TS)
            pltpu.make_async_copy(k_hbm.at[pl.ds(b, G), pl.ds(r0, TS), :],
                                  kbuf.at[slot, :, pl.ds(j * TS, TS), :], ksem.at[slot]).start(priority=0)
            pltpu.make_async_copy(v_hbm.at[pl.ds(b, G), pl.ds(r0, TS), :],
                                  vbuf.at[slot, :, pl.ds(j * TS, TS), :], vsem.at[slot]).start(priority=1)

    def wait_all(buf, sem):
        pltpu.make_async_copy(buf, buf, sem).wait()

    cx = pltpu.make_async_copy(x_hbm, x_v, wsem.at[5])
    cr = pltpu.make_async_copy(wr_hbm, wr_v, wsem.at[6])
    cq = pltpu.make_async_copy(wq_hbm, wq_v, wsem.at[0])
    co = pltpu.make_async_copy(wot_hbm, wot_v, wsem.at[1])
    cg = pltpu.make_async_copy(wg_hbm, wg_v, wsem.at[2])
    cu = pltpu.make_async_copy(wu_hbm, wu_v, wsem.at[3])
    cd = pltpu.make_async_copy(wdt_hbm, wdt_v, wsem.at[4])
    cx.start()
    cr.start()
    cq.start()
    for s in range(NBUF):
        issue(s, s)
        if s == 0:
            cg.start()
            cu.start()
            cd.start()
        if s == 1:
            co.start()

    cx.wait()
    x = x_v[0].astype(F32)
    mu = jnp.mean(x, axis=-1, keepdims=True)
    xc = x - mu
    var = jnp.mean(xc * xc, axis=-1, keepdims=True)
    xn = (xc * jax.lax.rsqrt(var + 1e-5)).astype(BF16).astype(F32)
    xn8 = jnp.broadcast_to(xn, (8, d)).astype(BF16)

    cq.wait()
    q = jnp.dot(xn8, wq_v[...], preferred_element_type=F32)
    q = q.astype(BF16).astype(F32) * (DH ** -0.5)
    row = jax.lax.broadcasted_iota(jnp.int32, (8, DH), 0)
    for g in range(hkv):
        qa = q[:, (2 * g) * DH:(2 * g + 1) * DH]
        qb = q[:, (2 * g + 1) * DH:(2 * g + 2) * DH]
        q_s[g] = jnp.where(row == 0, qa, qb)

    cg.wait()
    cu.wait()
    gate = jnp.dot(xn8, wg_v[...], preferred_element_type=F32).astype(BF16).astype(F32)
    up = jnp.dot(xn8, wu_v[...], preferred_element_type=F32).astype(BF16).astype(F32)
    hmid = (gate * jax.nn.sigmoid(gate) * up).astype(BF16)
    cd.wait()
    y = jax.lax.dot_general(hmid, wdt_v[...], NT, preferred_element_type=F32)[0:1]
    cr.wait()
    wr = wr_v[...].astype(F32).reshape(1, d)
    r = jnp.sum(xn * wr, axis=-1, keepdims=True)
    base = x + (xn + y * jax.nn.sigmoid(r))
    co.wait()

    def head_body(g, carry):
        acc_a, acc_b = carry
        qg = q_s[g].astype(BF16)

        def chunk_body(c, c2):
            m, l, acc = c2
            i = g * nc + c
            slot = i % NBUF
            wait_all(kbuf.at[slot], ksem.at[slot])
            s = jax.lax.dot_general(qg, kbuf[slot].reshape(T, DH), NT, preferred_element_type=F32)
            m_new = jnp.maximum(m, jnp.max(s, axis=-1, keepdims=True))
            alpha = jnp.exp(m - m_new)
            p = jnp.exp(s - m_new)
            l = alpha * l + jnp.sum(p, axis=-1, keepdims=True)
            wait_all(vbuf.at[slot], vsem.at[slot])
            acc = alpha * acc + jnp.dot(p.astype(BF16), vbuf[slot].reshape(T, DH), preferred_element_type=F32)

            @pl.when(i + NBUF < total)
            def _():
                issue(i + NBUF, slot)

            return m_new, l, acc

        m0 = jnp.full((8, 1), -jnp.inf, F32)
        l0 = jnp.zeros((8, 1), F32)
        a0 = jnp.zeros((8, DH), F32)
        _, l, acc = jax.lax.fori_loop(0, nc, chunk_body, (m0, l0, a0))
        o = (acc / l).astype(BF16)
        col = pl.multiple_of(g * (2 * DH), 2 * DH)
        acc_a = acc_a + jax.lax.dot_general(o, wot_v[:, pl.ds(col, DH)], NT, preferred_element_type=F32)
        acc_b = acc_b + jax.lax.dot_general(o, wot_v[:, pl.ds(col + DH, DH)], NT, preferred_element_type=F32)
        return acc_a, acc_b

    z = jnp.zeros((8, d), F32)
    acc_a, acc_b = jax.lax.fori_loop(0, hkv, head_body, (z, z))
    out_ref[0] = (base + (acc_a[0:1] + acc_b[1:2])).astype(out_ref.dtype)


@jax.jit
def pallas_parallel_sum__gqa_block_cached__moe_arch_mod__decode_kernel(
    A_x: jax.Array,
    A_k_cache: jax.Array,
    A_v_cache: jax.Array,
    A_wq: jax.Array,
    A_wo: jax.Array,
    B_x: jax.Array,
    B_w_r: jax.Array,
    B_w_gate: jax.Array,
    B_w_up: jax.Array,
    B_w_down: jax.Array,
):
    del B_x
    hkv = A_k_cache.shape[1]
    wot = A_wo.T
    wdt = B_w_down.T
    k3 = A_k_cache.reshape(-1, R, DH)
    v3 = A_v_cache.reshape(-1, R, DH)
    hbm = pl.BlockSpec(memory_space=pltpu.HBM)
    return pl.pallas_call(
        _kernel,
        out_shape=jax.ShapeDtypeStruct(A_x.shape, A_x.dtype),
        in_specs=[hbm] * 9,
        out_specs=pl.BlockSpec(memory_space=pltpu.VMEM),
        scratch_shapes=[
            pltpu.VMEM((NBUF, G, TT, DH), BF16),
            pltpu.VMEM((NBUF, G, TT, DH), BF16),
            pltpu.VMEM(A_x.shape, BF16),
            pltpu.VMEM(B_w_r.shape, BF16),
            pltpu.VMEM(A_wq.shape, BF16),
            pltpu.VMEM(wot.shape, BF16),
            pltpu.VMEM(B_w_gate.shape, BF16),
            pltpu.VMEM(B_w_up.shape, BF16),
            pltpu.VMEM(wdt.shape, BF16),
            pltpu.VMEM((hkv, 8, DH), F32),
            pltpu.SemaphoreType.DMA((NBUF,)),
            pltpu.SemaphoreType.DMA((NBUF,)),
            pltpu.SemaphoreType.DMA((7,)),
        ],
        compiler_params=pltpu.CompilerParams(vmem_limit_bytes=100 * 1024 * 1024),
    )(A_x, B_w_r, k3, v3, A_wq, wot, B_w_gate, B_w_up, wdt)
```

```python
import jax
import jax.numpy as jnp
from jax.experimental import pallas as pl
from jax.experimental.pallas import tpu as pltpu

HQ, DH = 16, 256
NT = (((1,), (1,)), ((), ()))

R = 2048
G = 8
TS = 8
ND = 16
TT = ND * TS
T = G * TT
NBUF = 4
F32, BF16 = jnp.float32, jnp.bfloat16


def _kernel(x_hbm, wr_hbm, k_hbm, v_hbm, wq_hbm, wot_hbm, wg_hbm, wu_hbm, wdt_hbm, out_ref,
            kbuf, vbuf, x_v, wr_v, wq_v, wot_v, wg_v, wu_v, wdt_v, q_s, h_s, ksem, vsem, wsem, dsem):
    hkv = q_s.shape[0]
    sk = k_hbm.shape[0] * R // hkv
    d = x_hbm.shape[-1]
    nc = sk // T
    nr = R // TT
    total = hkv * nc
    assert HQ == 2 * hkv and sk % (G * R) == 0 and total >= NBUF

    def issue(i, slot):
        b = pl.multiple_of((i // nr) * G, G)
        c = i % nr
        for j in range(ND):
            r0 = pl.multiple_of(c * TT + j * TS, TS)
            pltpu.make_async_copy(k_hbm.at[pl.ds(b, G), pl.ds(r0, TS), :],
                                  kbuf.at[slot, :, pl.ds(j * TS, TS), :], ksem.at[slot]).start(priority=0)
            pltpu.make_async_copy(v_hbm.at[pl.ds(b, G), pl.ds(r0, TS), :],
                                  vbuf.at[slot, :, pl.ds(j * TS, TS), :], vsem.at[slot]).start(priority=1)

    def wait_all(buf, sem):
        pltpu.make_async_copy(buf, buf, sem).wait()

    cx = pltpu.make_async_copy(x_hbm, x_v, wsem.at[5])
    cr = pltpu.make_async_copy(wr_hbm, wr_v, wsem.at[6])
    cq = pltpu.make_async_copy(wq_hbm, wq_v, wsem.at[0])
    co = pltpu.make_async_copy(wot_hbm, wot_v, wsem.at[1])
    cg = pltpu.make_async_copy(wg_hbm, wg_v, wsem.at[2])
    cu = pltpu.make_async_copy(wu_hbm, wu_v, wsem.at[3])

    def issue_wd():
        for j in range(d // 8):
            rows = pl.ds(j * 8, 8)
            pltpu.make_async_copy(wdt_hbm.at[rows], wdt_v.at[rows], dsem.at[j // 16]).start(priority=1)

    cx.start()
    cr.start()
    cq.start()
    for s in range(NBUF):
        issue(s, s)
        if s == 0:
            cg.start()
            cu.start()
        if s == 1:
            co.start()

    cx.wait()
    x = x_v[0].astype(F32)
    mu = jnp.mean(x, axis=-1, keepdims=True)
    xc = x - mu
    var = jnp.mean(xc * xc, axis=-1, keepdims=True)
    xn = (xc * jax.lax.rsqrt(var + 1e-5)).astype(BF16).astype(F32)
    xn8 = jnp.broadcast_to(xn, (8, d)).astype(BF16)

    cq.wait()
    q = jnp.dot(xn8, wq_v[...], preferred_element_type=F32)
    q = q.astype(BF16).astype(F32) * (DH ** -0.5)
    row = jax.lax.broadcasted_iota(jnp.int32, (8, DH), 0)
    for g in range(hkv):
        qa = q[:, (2 * g) * DH:(2 * g + 1) * DH]
        qb = q[:, (2 * g + 1) * DH:(2 * g + 2) * DH]
        q_s[g] = jnp.where(row == 0, qa, qb)

    cg.wait()
    cu.wait()
    gate = jnp.dot(xn8, wg_v[...], preferred_element_type=F32).astype(BF16).astype(F32)
    up = jnp.dot(xn8, wu_v[...], preferred_element_type=F32).astype(BF16).astype(F32)
    hmid = (gate * jax.nn.sigmoid(gate) * up).astype(BF16)
    h_s[...] = hmid
    cr.wait()
    wr = wr_v[...].astype(F32).reshape(1, d)
    r = jnp.sum(xn * wr, axis=-1, keepdims=True)
    r_sel = jax.nn.sigmoid(r)
    co.wait()

    def head_body(g, carry):
        acc_a, acc_b = carry
        qg = q_s[g].astype(BF16)

        def chunk_body(c, c2):
            m, l, acc = c2
            i = g * nc + c
            slot = i % NBUF
            wait_all(kbuf.at[slot], ksem.at[slot])
            s = jax.lax.dot_general(qg, kbuf[slot].reshape(T, DH), NT, preferred_element_type=F32)
            m_new = jnp.maximum(m, jnp.max(s, axis=-1, keepdims=True))
            alpha = jnp.exp(m - m_new)
            p = jnp.exp(s - m_new)
            ps = p[:, 0:128]
            for u in range(1, T // 128):
                ps = ps + p[:, u * 128:(u + 1) * 128]
            l = alpha * l + ps
            wait_all(vbuf.at[slot], vsem.at[slot])
            acc = alpha * acc + jnp.dot(p.astype(BF16), vbuf[slot].reshape(T, DH), preferred_element_type=F32)

            @pl.when(i + NBUF < total)
            def _():
                issue(i + NBUF, slot)

            @pl.when(i + NBUF == total)
            def _():
                issue_wd()

            return m_new, l, acc

        m0 = jnp.full((8, 1), -jnp.inf, F32)
        l0 = jnp.zeros((8, 128), F32)
        a0 = jnp.zeros((8, DH), F32)
        _, l, acc = jax.lax.fori_loop(0, nc, chunk_body, (m0, l0, a0))
        o = (acc / jnp.sum(l, axis=-1, keepdims=True)).astype(BF16)
        col = pl.multiple_of(g * (2 * DH), 2 * DH)
        acc_a = acc_a + jax.lax.dot_general(o, wot_v[:, pl.ds(col, DH)], NT, preferred_element_type=F32)
        acc_b = acc_b + jax.lax.dot_general(o, wot_v[:, pl.ds(col + DH, DH)], NT, preferred_element_type=F32)
        return acc_a, acc_b

    z = jnp.zeros((8, d), F32)
    acc_a, acc_b = jax.lax.fori_loop(0, hkv, head_body, (z, z))
    base = x + (acc_a[0:1] + acc_b[1:2]) + xn
    hm = h_s[...]
    ys = []
    for c in range(pl.cdiv(d, 128)):
        rows = slice(c * 128, min(d, (c + 1) * 128))
        wait_all(wdt_v.at[rows], dsem.at[c])
        ys.append(jax.lax.dot_general(hm, wdt_v[rows], NT, preferred_element_type=F32))
    y = jnp.concatenate(ys, axis=1)[0:1]
    out_ref[0] = (base + y * r_sel).astype(out_ref.dtype)


@jax.jit
def pallas_parallel_sum__gqa_block_cached__moe_arch_mod__decode_kernel(
    A_x: jax.Array,
    A_k_cache: jax.Array,
    A_v_cache: jax.Array,
    A_wq: jax.Array,
    A_wo: jax.Array,
    B_x: jax.Array,
    B_w_r: jax.Array,
    B_w_gate: jax.Array,
    B_w_up: jax.Array,
    B_w_down: jax.Array,
):
    del B_x
    hkv = A_k_cache.shape[1]
    wot = A_wo.T
    wdt = B_w_down.T
    k3 = A_k_cache.reshape(-1, R, DH)
    v3 = A_v_cache.reshape(-1, R, DH)
    hbm = pl.BlockSpec(memory_space=pltpu.HBM)
    return pl.pallas_call(
        _kernel,
        out_shape=jax.ShapeDtypeStruct(A_x.shape, A_x.dtype),
        in_specs=[hbm] * 9,
        out_specs=pl.BlockSpec(memory_space=pltpu.VMEM),
        scratch_shapes=[
            pltpu.VMEM((NBUF, G, TT, DH), BF16),
            pltpu.VMEM((NBUF, G, TT, DH), BF16),
            pltpu.VMEM(A_x.shape, BF16),
            pltpu.VMEM(B_w_r.shape, BF16),
            pltpu.VMEM(A_wq.shape, BF16),
            pltpu.VMEM(wot.shape, BF16),
            pltpu.VMEM(B_w_gate.shape, BF16),
            pltpu.VMEM(B_w_up.shape, BF16),
            pltpu.VMEM(wdt.shape, BF16),
            pltpu.VMEM((hkv, 8, DH), F32),
            pltpu.VMEM((8, wdt.shape[1]), BF16),
            pltpu.SemaphoreType.DMA((NBUF,)),
            pltpu.SemaphoreType.DMA((NBUF,)),
            pltpu.SemaphoreType.DMA((7,)),
            pltpu.SemaphoreType.DMA((4,)),
        ],
        compiler_params=pltpu.CompilerParams(vmem_limit_bytes=100 * 1024 * 1024,
                                             disable_bounds_checks=True),
    )(A_x, B_w_r, k3, v3, A_wq, wot, B_w_gate, B_w_up, wdt)
```
